```python
import os as _os
_os.environ.setdefault("JAX_PLATFORMS", "cpu")
import jax
import jax.numpy as jnp

def _softmax(x, axis=-1):
    return jax.nn.softmax(x, axis=axis)
def _gelu(x):
    return jax.nn.gelu(x, approximate=True)
def _silu(x):
    return jax.nn.silu(x)
def _sigmoid(x):
    return jax.nn.sigmoid(x)
def _layernorm(x, axis=-1, eps=1e-5):
    m = jnp.mean(x, axis=axis, keepdims=True)
    v = jnp.var(x, axis=axis, keepdims=True)
    return (x - m) / jnp.sqrt(v + eps)
def _scatter_add(tgt, idx, src, axis=0):
    return tgt.at[idx].add(src)
def _segment_sum(src, seg, n):
    return jax.ops.segment_sum(src, seg, n)
class _Rng:
    def __init__(self, key):
        self._k = key
    def _next(self):
        self._k, sub = jax.random.split(self._k)
        return sub
    def normal(self, shape):
        return jax.random.normal(self._next(), shape, dtype=jnp.bfloat16)
    def randint(self, lo, hi, shape):
        return jax.random.randint(self._next(), shape, lo, hi, dtype=jnp.int32)
    def uniform(self, shape, lo=0.0, hi=1.0):
        return jax.random.uniform(self._next(), shape, jnp.bfloat16, lo, hi)
    def permutation(self, n):
        return jax.random.permutation(self._next(), n)


kernel_name = 'sequential_preLN__linear_attn_block__glu_gated_reglu__prompt'

def setup_inputs():
    _rng = _Rng(jax.random.key(int.from_bytes(__import__("os").urandom(4), "little")))
    _w = (lambda a: (lambda t: t.astype(jnp.bfloat16) if jnp.issubdtype(t.dtype, jnp.floating) else t)(jnp.asarray(a)))
    def _A_setup():
        B, S, D = 1, 2048, 640
        return {
            "x": _w((lambda *s: _rng.normal(s) * 0.05)(B, S, D)),
            "wqkv": _w((lambda *s: _rng.normal(s) * 0.05)(D, 3 * D)),
            "wo": _w((lambda *s: _rng.normal(s) * 0.05)(D, D)),
        }
    _A_in = _A_setup()

    def _B_setup():
        B, S, D, F = 1, 2048, 640, 1536
        return {
            "x": _w((lambda *s: _rng.normal(s) * 0.05)(B, S, D)),
            "W_gate": _w((lambda *s: _rng.normal(s) * 0.05)(D, F) * (2.0 / D) ** 0.5),
            "W_up": _w((lambda *s: _rng.normal(s) * 0.05)(D, F) * (2.0 / D) ** 0.5),
            "W_down": _w((lambda *s: _rng.normal(s) * 0.05)(F, D) * (1.0 / F) ** 0.5),
        }
    _B_in = _B_setup()

    return {
        "A_x": _A_in["x"],
        "A_wqkv": _A_in["wqkv"],
        "A_wo": _A_in["wo"],
        "B_x": _B_in["x"],
        "B_W_gate": _B_in["W_gate"],
        "B_W_up": _B_in["W_up"],
        "B_W_down": _B_in["W_down"],
    }

def reference(A_x, A_wqkv, A_wo, B_x, B_W_gate, B_W_up, B_W_down):
    def _A_ref(x, wqkv, wo):
        B, S, D = x.shape
        H = 32; Dh = D // H
        qkv = (lambda x, *d: x.transpose(*d))((x @ wqkv).reshape(B, S, 3, H, Dh), 2, 0, 3, 1, 4)
        q, k, v = qkv[0], qkv[1], qkv[2]
        phi = lambda t: jnp.where(t > 0, t + 1, jnp.exp(t)) + 1e-6
        pq, pk = phi(q), phi(k)
        kv = jnp.einsum("bhsd,bhse->bhde", pk, v)
        z = jnp.einsum("bhsd->bhd", pk)
        num = jnp.einsum("bhqd,bhde->bhqe", pq, kv)
        den = jnp.einsum("bhqd,bhd->bhq", pq, z)[..., None] + 1e-6
        o = num / den
        return (lambda x, *d: x.transpose(*d))(o, 0, 2, 1, 3).reshape(B, S, D) @ wo

    def _B_ref(x, W_gate, W_up, W_down):
        gate = jnp.einsum("bsd,df->bsf", x, W_gate)
        up = jnp.einsum("bsd,df->bsf", x, W_up)
        gate = gate * (lambda x, dt: x.astype(dt))(gate > 0, gate.dtype)
        h = gate * up
        return jnp.einsum("bsf,fd->bsd", h, W_down)

    x = A_x
    h = x + _A_ref(_layernorm(x, axis=-1), A_wqkv, A_wo)
    h2 = h + _B_ref(_layernorm(h, axis=-1), B_W_gate, B_W_up, B_W_down)
    return h2
```

```python
import functools
import jax
import jax.numpy as jnp
import numpy as np
from jax import lax
import jax.experimental.pallas as pl
import jax.experimental.pallas.tpu as pltpu

S, D, H, DH, F = 2048, 640, 32, 20, 1536
f32, bf16 = jnp.float32, jnp.bfloat16
NT = (((1,), (1,)), ((), ()))
NL = D // 128


def _ln(x):
    m = jnp.mean(x, axis=-1, keepdims=True)
    xc = x - m
    v = jnp.mean(xc * xc, axis=-1, keepdims=True)
    return xc * lax.rsqrt(v + 1e-5)


def _ln2(x):
    m = jnp.mean(x, axis=-1, keepdims=True)
    xc = x - m
    v = jnp.mean(xc * xc, axis=-1, keepdims=True)
    rs = lax.rsqrt(v + 1e-5)
    return xc * rs, rs


def _phi(t):
    return jnp.where(t > 0, t + 1.0, jnp.exp(t)) + 1e-6


def _kernel(x_hbm, wqkv_hbm, wo_hbm, wg_hbm, wu_hbm, wd_hbm, o_hbm,
            x_v, xn_v, wq_v, wk_v, wv_v, wo_v, wg_v, wu_v, wd_v,
            wkT_v, wqTp_v, tmp_v, wvT_v, g_v, z_v, mp_v, o_v, h_v, hn_v, r_v, mask_v, act_v,
            xsem, wsem, osem, *, TM1, TM2, FC, order, jmode, RC, TAIL, GP, QG):
    n1 = len(TM1)
    O1 = [sum(TM1[:i]) for i in range(n1)]
    assert sum(TM1) == S
    n2 = S // TM2
    nc = F // FC

    xc = [pltpu.make_async_copy(x_hbm.at[pl.ds(O1[i], TM1[i])], x_v.at[pl.ds(O1[i], TM1[i])], xsem.at[i]) for i in range(n1)]
    wc = dict(
        k=pltpu.make_async_copy(wqkv_hbm.at[:, pl.ds(D, D)], wk_v, wsem.at[0]),
        q=pltpu.make_async_copy(wqkv_hbm.at[:, pl.ds(0, D)], wq_v, wsem.at[1]),
        v=pltpu.make_async_copy(wqkv_hbm.at[:, pl.ds(2 * D, D)], wv_v, wsem.at[2]),
        o=pltpu.make_async_copy(wo_hbm, wo_v, wsem.at[3]),
        g=pltpu.make_async_copy(wg_hbm, wg_v, wsem.at[4]),
        u=pltpu.make_async_copy(wu_hbm, wu_v, wsem.at[5]),
        d=pltpu.make_async_copy(wd_hbm, wd_v, wsem.at[6]),
    )
    oc = [pltpu.make_async_copy(o_v.at[pl.ds(j * TM2, TM2)], o_hbm.at[pl.ds(j * TM2, TM2)], osem.at[j]) for j in range(n2 - 1)]
    oc += [pltpu.make_async_copy(o_v.at[pl.ds(S - TM2, TM2), pl.ds(c0, c1 - c0)], o_hbm.at[pl.ds(S - TM2, TM2), pl.ds(c0, c1 - c0)], osem.at[n2 - 1 + pi]) for pi, (c0, c1) in enumerate(TAIL)]
    st = {}

    def permute_rows(val, dst):
        for a in range(NL):
            tmp_v[a] = val[:, a * 128:(a + 1) * 128]
        for a in range(NL):
            for d in range(DH):
                dst[pl.ds(d * H, H), a * 128:(a + 1) * 128] = tmp_v[a, pl.ds(d, H, stride=DH), :].astype(bf16)

    def L(i):
        for r0 in range(O1[i], O1[i] + TM1[i], RC):
            r = pl.ds(r0, RC)
            xn_v[r, :] = _ln(x_v[r, :].astype(f32)).astype(bf16)

    def WK():
        wkT_v[...] = wk_v[...].astype(f32).T.astype(bf16)

    def WQ():
        permute_rows(wq_v[...].astype(f32).T, wqTp_v)

    def WV():
        ri = lax.broadcasted_iota(jnp.int32, (120, 128), 0) // DH
        ci = lax.broadcasted_iota(jnp.int32, (120, 128), 1) // DH
        mask_v[...] = jnp.where(ri == ci, 1.0, 0.0)
        if jmode == 'ha':
            wvT_v[...] = wv_v[...].astype(f32).T

    def K(i):
        xn = xn_v[pl.ds(O1[i], TM1[i]), :]
        kT = lax.dot_general(wkT_v[...], xn, NT, preferred_element_type=f32)
        pkT = _phi(kT)
        zs = pkT[:, 0:128]
        for t in range(1, TM1[i] // 128):
            zs = zs + pkT[:, t * 128:(t + 1) * 128]
        st['z'] = zs if i == 0 else st['z'] + zs
        st['pk', i] = pkT.astype(bf16)

    def G(i):
        xn = xn_v[pl.ds(O1[i], TM1[i]), :]
        g = jnp.dot(st.pop(('pk', i)), xn, preferred_element_type=f32)
        st['g'] = g if i == 0 else st['g'] + g

    def Z():
        z_v[...] = st.pop('z')
        zperm = jnp.concatenate([z_v[pl.ds(d, H, stride=DH), :] for d in range(DH)], axis=0)
        st['zrow'] = jnp.sum(zperm.T, axis=0, keepdims=True)

    def blocks_for_tile(a):
        lo = (a * 128 // DH) * DH
        hi = -(-((a + 1) * 128) // DH) * DH
        return lo // 128, min(NL, -(-hi // 128))

    def J1():
        g = st.pop('g')
        if jmode == 'full':
            kv = jnp.dot(g.astype(bf16), wv_v[...], preferred_element_type=f32)
            ri = lax.broadcasted_iota(jnp.int32, (D, D), 0) // DH
            ci = lax.broadcasted_iota(jnp.int32, (D, D), 1) // DH
            st['kv'] = jnp.where(ri == ci, kv, 0.0).astype(bf16)
        elif jmode == 'tri':
            out = []
            for a in range(NL):
                lo, hi = blocks_for_tile(a)
                kv = jnp.dot(g[a * 128:(a + 1) * 128].astype(bf16), wv_v[:, lo * 128:hi * 128], preferred_element_type=f32)
                w = (hi - lo) * 128
                ri = (lax.broadcasted_iota(jnp.int32, (128, w), 0) + a * 128) // DH
                ci = (lax.broadcasted_iota(jnp.int32, (128, w), 1) + lo * 128) // DH
                out.append(jnp.where(ri == ci, kv, 0.0).astype(bf16))
            st['kv'] = out
        else:
            g_v[...] = g
            out = []
            for r0 in range(0, D, 120):
                n = min(120, D - r0)
                kv = lax.dot_general(g_v[pl.ds(r0, n), :].astype(bf16), wvT_v[pl.ds(r0, n), :].astype(bf16), NT, preferred_element_type=f32)
                out.append(jnp.where(mask_v[0:n, 0:n] > 0, kv, 0.0).astype(bf16))
            st['kv'] = out

    def J2():
        kv = st.pop('kv')
        if jmode == 'full':
            m = jnp.dot(kv, wo_v[...], preferred_element_type=f32)
        elif jmode == 'tri':
            ms = []
            for a in range(NL):
                lo, hi = blocks_for_tile(a)
                ms.append(jnp.dot(kv[a], wo_v[lo * 128:hi * 128, :], preferred_element_type=f32))
            m = jnp.concatenate(ms, axis=0)
        else:
            ms = []
            tmpf = wo_v[...].astype(f32)
            for gi, r0 in enumerate(range(0, D, 120)):
                n = min(120, D - r0)
                ms.append(jnp.dot(kv[gi], tmpf[r0:r0 + n].astype(bf16), preferred_element_type=f32))
            m = jnp.concatenate(ms, axis=0)
        permute_rows(m, mp_v)

    def Q(j):
        xn = xn_v[pl.ds(j * TM2, TM2), :]
        pq = _phi(lax.dot_general(xn, wqTp_v[...], NT, preferred_element_type=f32))
        def epi(pq):
            t = pq * st['zrow']
            u = t[:, 0:128]
            for a in range(1, NL):
                u = u + t[:, a * 128:(a + 1) * 128]
            u = u + pltpu.roll(u, 64, 1)
            u = u + pltpu.roll(u, 32, 1)
            inv = 1.0 / (u + 1e-6)
            return (pq * jnp.concatenate([inv] * NL, axis=1)).astype(bf16), inv
        if QG == 0:
            r_v[pl.ds(j * TM2, TM2), :] = epi(pq)[0]
        else:
            h_v[pl.ds(j * TM2, TM2), :] = pq
            gates = [None] * QG
            for ci, r0 in enumerate(range(j * TM2, (j + 1) * TM2, RC)):
                p = h_v[pl.ds(r0, RC), :]
                if gates[ci % QG] is not None:
                    p = p + gates[ci % QG]
                r, inv = epi(p)
                gates[ci % QG] = jnp.where(inv[:, 0:1] < 0, 1.0, 0.0)
                r_v[pl.ds(r0, RC), :] = r

    def A(j):
        rows = pl.ds(j * TM2, TM2)
        a = jnp.dot(r_v[rows, :], mp_v[...], preferred_element_type=f32)
        h_v[rows, :] = x_v[rows, :].astype(f32) + a
        gates = st.setdefault('gates', [None] * GP)
        for ci, r0 in enumerate(range(j * TM2, (j + 1) * TM2, RC)):
            hh = h_v[pl.ds(r0, RC), :]
            if gates[ci % GP] is not None:
                hh = hh + gates[ci % GP]
            y, rs = _ln2(hh)
            if GP < 50:
                gates[ci % GP] = jnp.where(rs < 0, 1.0, 0.0)
            hn_v[pl.ds(r0, RC), :] = y.astype(bf16)

    def WF():
        wc['g'].wait()
        wc['u'].wait()

    def Y(j, c):
        hn = hn_v[pl.ds(j * TM2, TM2), :]
        cs = slice(c * FC, (c + 1) * FC)
        g = jnp.dot(hn, wg_v[:, cs], preferred_element_type=f32)
        up = jnp.dot(hn, wu_v[:, cs], preferred_element_type=f32)
        act = (jnp.maximum(g, 0.0) * up).astype(bf16)
        prev = h_v[pl.ds(j * TM2, TM2), :] if c == 0 else st['acc', j]
        if c < nc - 1:
            st['acc', j] = prev + jnp.dot(act, wd_v[cs, :], preferred_element_type=f32)
        elif j < n2 - 1:
            o_v[pl.ds(j * TM2, TM2), :] = (prev + jnp.dot(act, wd_v[cs, :], preferred_element_type=f32)).astype(bf16)
            oc[j].start()
        else:
            for pi, (c0, c1) in enumerate(TAIL):
                o_v[pl.ds(j * TM2, TM2), c0:c1] = (prev[:, c0:c1] + jnp.dot(act, wd_v[cs, c0:c1], preferred_element_type=f32)).astype(bf16)
                oc[j + pi].start()

    def Yu(j, c):
        hn = hn_v[pl.ds(j * TM2, TM2), :]
        cs = slice(c * FC, (c + 1) * FC)
        g = jnp.dot(hn, wg_v[:, cs], preferred_element_type=f32)
        up = jnp.dot(hn, wu_v[:, cs], preferred_element_type=f32)
        act_v[j % 2, :, cs] = (jnp.maximum(g, 0.0) * up).astype(bf16)

    def Yd(j):
        rows = pl.ds(j * TM2, TM2)
        if j < n2 - 1:
            o_v[rows, :] = (h_v[rows, :] + jnp.dot(act_v[j % 2], wd_v[...], preferred_element_type=f32)).astype(bf16)
            oc[j].start()
        else:
            for pi, (c0, c1) in enumerate(TAIL):
                o_v[rows, c0:c1] = (h_v[rows, c0:c1] + jnp.dot(act_v[j % 2], wd_v[:, c0:c1], preferred_element_type=f32)).astype(bf16)
                oc[j + pi].start()

    def X():
        g_v[...] = st.pop('g')

    def D0():
        xc[0].start(); wc['k'].start()

    def D1():
        for i in range(1, n1):
            xc[i].start()
        wc['q'].start()

    def D2():
        wc['v'].start(); wc['o'].start()

    def D3():
        wc['g'].start(); wc['u'].start(); wc['d'].start()

    fns = dict(L=L, WK=WK, WQ=WQ, WV=WV, WF=WF, K=K, G=G, Z=Z, Ja=J1, Jb=J2, X=X, Q=Q, A=A, Y=Y, Yu=Yu, Yd=Yd, Da=D0, Db=D1, Dc=D2, Dd=D3)
    for tok in order.split():
        if tok[0] in 'ws' and tok[1:] in wc:
            wc[tok[1:]].wait() if tok[0] == 'w' else wc[tok[1:]].start()
            continue
        if tok[:2] in ('wx', 'sx'):
            xc[int(tok[2:])].wait() if tok[0] == 'w' else xc[int(tok[2:])].start()
            continue
        name = tok.rstrip('0123456789,')
        args = tok[len(name):]
        args = [int(a) for a in args.split(',')] if args else []
        fns[name](*args)
    for c in (oc if 'Yd3' in order or 'Y3,2' in order else []):
        c.wait()


T = "Y0,0 Y0,1 Y0,2 Y1,0 Y1,1 Y1,2 Y2,0 Y2,1 Y2,2 Y3,0 Y3,1 Y3,2"
ORD = ("sx0 sk sx1 sx2 wx0 L0 wk wx1 sq sx3 sx4 sv so sg su sd WK K0 L1 K1 G0 wx2 L2 G1 K2 wq wx3 wx4 wv wo L3 WQ G2 K3 L4 WV K4 G3 Z Q0 G4 wg wu wd Q1 Ja Q2 Jb Q3 A0 A1 A2 A3 " + T)

def build(TM1=(256,256,512,512,512), TM2=512, FC=512, order=ORD, jmode='ha', RC=32, GP=1, QG=0, TAIL=((0, 384), (384, 512), (512, 640)), interpret=False):
    kern = functools.partial(_kernel, TM1=TM1, TM2=TM2, FC=FC, order=order, jmode=jmode, RC=RC, TAIL=TAIL, GP=GP, QG=QG)

    @jax.jit
    def run(A_x, A_wqkv, A_wo, B_x, B_W_gate, B_W_up, B_W_down):
        x2 = A_x.reshape(S, D)
        anyspec = pl.BlockSpec(memory_space=pl.ANY)
        out = pl.pallas_call(
            kern,
            in_specs=[anyspec] * 6,
            out_specs=anyspec,
            out_shape=jax.ShapeDtypeStruct((S, D), bf16),
            scratch_shapes=[
                pltpu.VMEM((S, D), bf16),
                pltpu.VMEM((S, D), bf16),
                pltpu.VMEM((D, D), bf16),
                pltpu.VMEM((D, D), bf16),
                pltpu.VMEM((D, D), bf16),
                pltpu.VMEM((D, D), bf16),
                pltpu.VMEM((D, F), bf16),
                pltpu.VMEM((D, F), bf16),
                pltpu.VMEM((F, D), bf16),
                pltpu.VMEM((D, D), bf16),
                pltpu.VMEM((D, D), bf16),
                pltpu.VMEM((NL, D, 128), f32),
                pltpu.VMEM((D, D), f32),
                pltpu.VMEM((D, D), f32),
                pltpu.VMEM((D, 128), f32),
                pltpu.VMEM((D, D), bf16),
                pltpu.VMEM((S, D), bf16),
                pltpu.VMEM((S, D), f32),
                pltpu.VMEM((S, D), bf16),
                pltpu.VMEM((S, D), bf16),
                pltpu.VMEM((120, 128), f32),
                pltpu.VMEM((2, TM2, F), bf16),
                pltpu.SemaphoreType.DMA((len(TM1),)),
                pltpu.SemaphoreType.DMA((7,)),
                pltpu.SemaphoreType.DMA((S // TM2 + len(TAIL),)),
            ],
            compiler_params=pltpu.CompilerParams(vmem_limit_bytes=100 * 1024 * 1024),
            interpret=interpret,
        )(x2, A_wqkv, A_wo, B_W_gate, B_W_up, B_W_down)
        return out.reshape(1, S, D)

    return run


_RUN = build(**dict(TM1=(256, 256, 512, 512, 512),GP=1,RC=16,order='sx0 sk sx1 wx0 L0 wk wx1 sx2 sq sx3 sx4 sv so WK L1 K0 K1 G0 wx2 L2 G1 K2 wq wx3 wx4 wo wv L3 sg G2 su L4 sd WQ K3 K4 G3 Z Q0 WV G4 Ja Jb wg wu wd Q2 Q1 A0 A1 Q3 A2 Yu0,2 Yu0,0 Yu1,1 Yu0,1 Yd0 Yu1,2 A3 Yu2,0 Yu1,0 Yd1 Yu2,1 Yu2,2 Yd2 Yu3,0 Yu3,1 Yu3,2 Yd3'))


def pallas_sequential_preLN__linear_attn_block__glu_gated_reglu__prompt_kernel(
        A_x, A_wqkv, A_wo, B_x, B_W_gate, B_W_up, B_W_down):
    return _RUN(A_x, A_wqkv, A_wo, B_x, B_W_gate, B_W_up, B_W_down)
```
